```python
import os as _os
_os.environ.setdefault("JAX_PLATFORMS", "cpu")
import jax
import jax.numpy as jnp

def _softmax(x, axis=-1):
    return jax.nn.softmax(x, axis=axis)
def _gelu(x):
    return jax.nn.gelu(x, approximate=True)
def _silu(x):
    return jax.nn.silu(x)
def _sigmoid(x):
    return jax.nn.sigmoid(x)
def _layernorm(x, axis=-1, eps=1e-5):
    m = jnp.mean(x, axis=axis, keepdims=True)
    v = jnp.var(x, axis=axis, keepdims=True)
    return (x - m) / jnp.sqrt(v + eps)
def _scatter_add(tgt, idx, src, axis=0):
    return tgt.at[idx].add(src)
def _segment_sum(src, seg, n):
    return jax.ops.segment_sum(src, seg, n)
class _Rng:
    def __init__(self, key):
        self._k = key
    def _next(self):
        self._k, sub = jax.random.split(self._k)
        return sub
    def normal(self, shape):
        return jax.random.normal(self._next(), shape, dtype=jnp.bfloat16)
    def randint(self, lo, hi, shape):
        return jax.random.randint(self._next(), shape, lo, hi, dtype=jnp.int32)
    def uniform(self, shape, lo=0.0, hi=1.0):
        return jax.random.uniform(self._next(), shape, jnp.bfloat16, lo, hi)
    def permutation(self, n):
        return jax.random.permutation(self._next(), n)


kernel_name = 'sequential_preLN__sliding_local_dilated__dense_activation_relu__prompt'

def setup_inputs():
    _rng = _Rng(jax.random.key(int.from_bytes(__import__("os").urandom(4), "little")))
    _w = (lambda a: (lambda t: t.astype(jnp.bfloat16) if jnp.issubdtype(t.dtype, jnp.floating) else t)(jnp.asarray(a)))
    def _A_setup():
        B, S, D = 1, 2048, 1024
        return {
            "x": _w((lambda *s: _rng.normal(s) * 0.05)(B, S, D)),
            "wqkv": _w((lambda *s: _rng.normal(s) * 0.05)(D, 3 * D)),
            "wo": _w((lambda *s: _rng.normal(s) * 0.05)(D, D)),
        }
    _A_in = _A_setup()

    def _B_setup():
        B, S, D, Dff = 1, 2048, 1024, 3584
        return {
            "x": _w((lambda *s: _rng.normal(s) * 0.05)(B, S, D)),
            "w1": _w((lambda *s: _rng.normal(s) * 0.05)(D, Dff)),
            "w2": _w((lambda *s: _rng.normal(s) * 0.05)(Dff, D)),
        }
    _B_in = _B_setup()

    return {
        "A_x": _A_in["x"],
        "A_wqkv": _A_in["wqkv"],
        "A_wo": _A_in["wo"],
        "B_x": _B_in["x"],
        "B_w1": _B_in["w1"],
        "B_w2": _B_in["w2"],
    }

def reference(A_x, A_wqkv, A_wo, B_x, B_w1, B_w2):
    def _A_ref(x, wqkv, wo):
        B, S, D = x.shape
        H = 32; Dh = D // H
        W, dil = 8, 2
        qkv = (lambda x, *d: x.transpose(*d))((x @ wqkv).reshape(B, S, 3, H, Dh), 2, 0, 3, 1, 4)
        q, k, v = qkv[0], qkv[1], qkv[2]
        scale = Dh ** -0.5
        pos = jnp.arange(S)
        off = jnp.arange(W) * dil
        idx = pos[:, None] - off[None, :]
        mask = idx >= 0
        idx_c = jnp.where(mask, idx, 0).reshape(-1)
        kg = k[:, :, idx_c, :].reshape(B, H, S, W, Dh)
        vg = v[:, :, idx_c, :].reshape(B, H, S, W, Dh)
        logits = jnp.einsum("bhsd,bhswd->bhsw", q, kg) * scale
        logits = jnp.where(mask[None, None, :, :], logits, -1e9)
        attn = _softmax(logits, axis=-1)
        o = jnp.einsum("bhsw,bhswd->bhsd", attn, vg)
        return (lambda x, *d: x.transpose(*d))(o, 0, 2, 1, 3).reshape(B, S, D) @ wo

    def _B_ref(x, w1, w2):
        h = jnp.einsum("bsd,df->bsf", x, w1)
        zero = jnp.zeros_like(h)
        h = jnp.maximum(h, zero)
        return jnp.einsum("bsf,fd->bsd", h, w2)

    x = A_x
    h = x + _A_ref(_layernorm(x, axis=-1), A_wqkv, A_wo)
    h2 = h + _B_ref(_layernorm(h, axis=-1), B_w1, B_w2)
    return h2
```

```python
import functools
import jax
import jax.numpy as jnp
from jax import lax
import jax.experimental.pallas as pl
import jax.experimental.pallas.tpu as pltpu

H = 32
WIN = 8
DIL = 2
HALO = 16
EPS = 1e-5
F32 = jnp.float32
BF16 = jnp.bfloat16


def _ln(x):
    m = jnp.mean(x, axis=-1, keepdims=True)
    xc = x - m
    v = jnp.mean(xc * xc, axis=-1, keepdims=True)
    return xc * lax.rsqrt(v + EPS)


def _kernel(x_hbm, wqkv_hbm, wo_hbm, w1_hbm, w2_hbm, o_ref,
            wraw_scr, wt_scr, stage_scr, wo_scr, w1_scr, w2_scr,
            qkv_scr, att_scr, h_scr, ln2_scr, h1_scr, ln1_scr, x_scr, sems, *, TS, D, F, FC, NC, NT, R1, R2):
    i = pl.program_id(0)
    Dh = D // H
    scale = Dh ** -0.5
    NV = D // 128
    G = 128 // H
    NF = F // FC
    NN = D // NC
    SS = Dh + 1

    def cp_qkv(p):
        return pltpu.make_async_copy(
            wqkv_hbm.at[:, pl.ds(pl.multiple_of(p * D, D), D)], wraw_scr.at[p], sems.at[p])

    def cp_wo():
        return pltpu.make_async_copy(wo_hbm, wraw_scr.at[3], sems.at[3])

    def cp_w1(f):
        return pltpu.make_async_copy(
            w1_hbm.at[:, pl.ds(pl.multiple_of(f * FC, FC), FC)], w1_scr.at[f], sems.at[4 + f])

    def cp_w2(n):
        return pltpu.make_async_copy(
            w2_hbm.at[:, pl.ds(pl.multiple_of(n * NC, NC), NC)], w2_scr.at[n], sems.at[4 + NF + n])

    XS = 4 + NF + NN

    def cp_x0():
        return pltpu.make_async_copy(x_hbm.at[pl.ds(0, TS), :], x_scr.at[pl.ds(0, TS), :], sems.at[XS])

    def cp_x1():
        return pltpu.make_async_copy(x_hbm.at[pl.ds(TS, TS), :], x_scr.at[pl.ds(TS, TS), :], sems.at[XS + 1])

    def cp_x2():
        return pltpu.make_async_copy(x_hbm.at[pl.ds(2 * TS, TS), :], x_scr.at[pl.ds(2 * TS, TS), :], sems.at[XS + 2])

    def cp_xr():
        n = (NT - 3) * TS
        return pltpu.make_async_copy(x_hbm.at[pl.ds(3 * TS, n), :], x_scr.at[pl.ds(3 * TS, n), :], sems.at[XS + 3])

    x_ref = x_scr.at[pl.ds(pl.multiple_of(jnp.minimum(i, NT - 1) * TS, TS), TS), :]
    xn_ref = x_scr.at[pl.ds(pl.multiple_of(jnp.minimum(i + 1, NT - 1) * TS, TS), TS), :]

    def perm_base(d):
        return (d // G) * 128 + (d % G) * H

    def att_rows(r0, nrows, masked, pre=None):
        RC = 16
        dep = None
        sc = scale if pre is None else scale + jnp.where(i < 0, pre, 0.0)
        for c in range(nrows // RC):
            rr = r0 + c * RC
            q = [qkv_scr[j, pl.ds(HALO + rr, RC), :] * sc for j in range(NV)]
            logits = []
            for w in range(WIN):
                acc = None
                for j in range(NV):
                    kk = qkv_scr[NV + j, pl.ds(HALO + rr - DIL * w, RC), :]
                    t = q[j] * kk
                    acc = t if acc is None else acc + t
                acc = acc + pltpu.roll(acc, 64, 1)
                acc = acc + pltpu.roll(acc, 32, 1)
                if masked and w > 0:
                    row = rr + lax.broadcasted_iota(jnp.int32, (RC, 128), 0)
                    acc = jnp.where(row >= DIL * w, acc, -1e9)
                logits.append(acc)
            m = logits[0]
            for w in range(1, WIN):
                m = jnp.maximum(m, logits[w])
            es = [jnp.exp(l - m) for l in logits]
            den = es[0]
            for w in range(1, WIN):
                den = den + es[w]
            inv = 1.0 / den
            ps = [e * inv for e in es]
            for j in range(NV):
                acc = None
                for w in range(WIN):
                    vv = qkv_scr[2 * NV + j, pl.ds(HALO + rr - DIL * w, RC), :]
                    t = ps[w] * vv
                    acc = t if acc is None else acc + t
                att_scr[pl.ds(rr, RC), pl.ds(j * 128, 128)] = acc.astype(BF16)
                dep = acc if dep is None else dep + acc
        return dep

    def ln_rows(src_ref, dst_ref, pre=None):
        RC = 16
        dep = None
        for c in range(TS // RC):
            xx = src_ref[pl.ds(c * RC, RC), :].astype(F32)
            m = jnp.mean(xx, axis=-1, keepdims=True)
            if pre is not None:
                m = m + jnp.where(i < 0, pre[:, 0:1], 0.0)
            xc = xx - m
            v = jnp.mean(xc * xc, axis=-1, keepdims=True)
            y = xc * lax.rsqrt(v + EPS)
            dst_ref[pl.ds(c * RC, RC), :] = y.astype(BF16)
            for j in range(NV):
                t = y[:, j * 128:(j + 1) * 128]
                dep = t if dep is None else dep + t
        return dep

    def tie(lhs, dep):
        if dep is None:
            return lhs
        z = jnp.where(i < 0, dep, 0.0).astype(lhs.dtype)
        top = lhs[0:16, :]
        top = jnp.concatenate([top[:, 0:128] + z, top[:, 128:]], axis=1)
        return jnp.concatenate([top, lhs[16:, :]], axis=0)

    @pl.when(i == 0)
    def _():
        cp_x0().start()
        for p in range(3):
            cp_qkv(p).start()
        cp_wo().start()
        cp_x1().start()
        cp_x2().start()
        for f in range(NF):
            cp_w1(f).start()
        for n in range(NN):
            cp_w2(n).start()
        cp_xr().start()
        qkv_scr[:, pl.ds(0, HALO), :] = jnp.zeros((3 * NV, HALO, 128), F32)
        cp_x0().wait()

        ln1_scr[...] = _ln(x_ref[...].astype(F32)).astype(BF16)

        def prep_qkv(p, carry):
            cp_qkv(p).wait()
            for kb in range(NV):
                blk = wraw_scr[p, pl.ds(kb * 128, 128), :].astype(F32)
                blkt = blk.T
                for hh in range(H):
                    stage_scr[kb, pl.ds(hh * SS, Dh), :] = blkt[hh * Dh:(hh + 1) * Dh, :]
                for d in range(Dh):
                    rows = stage_scr[kb, pl.ds(d, H, stride=SS), :]
                    wt_scr[p, pl.ds(perm_base(d), H), pl.ds(kb * 128, 128)] = rows.astype(BF16)
            res = lax.dot_general(ln1_scr[...], wt_scr[p], (((1,), (1,)), ((), ())),
                                  preferred_element_type=F32)
            for j in range(NV):
                qkv_scr[p * NV + j, pl.ds(HALO, TS), :] = res[:, j * 128:(j + 1) * 128]
            return carry

        lax.fori_loop(0, 3, prep_qkv, 0)
        cp_wo().wait()

        def prep_wo(kb, carry):
            k0 = pl.multiple_of(kb * 128, 128)
            blkt = wraw_scr[3, :, pl.ds(k0, 128)].astype(F32)
            for hh in range(H):
                stage_scr[0, pl.ds(hh * SS, Dh), :] = blkt[hh * Dh:(hh + 1) * Dh, :]
            for d in range(Dh):
                rows = stage_scr[0, pl.ds(d, H, stride=SS), :]
                wo_scr[pl.ds(perm_base(d), H), pl.ds(k0, 128)] = rows.astype(BF16)
            return carry

        lax.fori_loop(0, NV, prep_wo, 0)
        cp_x1().wait()
        ln1_scr[...] = _ln(xn_ref[...].astype(F32)).astype(BF16)

    @pl.when(jnp.logical_and(i > 0, i < NT))
    def _():
        qkv_scr[:, pl.ds(0, HALO), :] = qkv_scr[:, pl.ds(TS, HALO), :]

    @pl.when(jnp.logical_and(i > 0, i < NT))
    def _():
        dep = None
        for p in range(3):
            res = lax.dot_general(tie(ln1_scr[...], dep), wt_scr[p], (((1,), (1,)), ((), ())),
                                  preferred_element_type=F32)
            for j in range(NV):
                qkv_scr[p * NV + j, pl.ds(HALO, TS), :] = res[:, j * 128:(j + 1) * 128]
            dep = ln_rows(h_scr, ln2_scr) if p == 0 else None

    @pl.when(i == NT)
    def _():
        ln2_scr[...] = _ln(h_scr[...]).astype(BF16)

    @pl.when(i == 0)
    def _():
        def body(r, carry):
            att_rows(pl.multiple_of(r * 16, 16), 16, True)
            return carry
        lax.fori_loop(0, TS // 16, body, 0)

    @pl.when(i == 1)
    def _():
        for f in range(NF):
            cp_w1(f).wait()
        for n in range(NN):
            cp_w2(n).wait()
        cp_x2().wait()

    @pl.when(i == 2)
    def _():
        cp_xr().wait()

    @pl.when(i > 0)
    def _():
        dep = None
        pre = None
        for f in range(NF):
            h1 = jnp.dot(tie(ln2_scr[...], dep), w1_scr[f], preferred_element_type=F32)
            h1_scr[:, pl.ds(f * FC, FC)] = jnp.maximum(h1, 0.0).astype(BF16)
            dep = att_rows(f * R1, R1, False, pre)
            pre = h1[TS - 16:, FC - 128:]
        for n in range(NN):
            c0 = n * NC
            t = jnp.dot(tie(h1_scr[...], dep), w2_scr[n], preferred_element_type=F32)
            o_ref[:, pl.ds(c0, NC)] = (
                h_scr[:, pl.ds(c0, NC)] + t.astype(BF16).astype(F32)).astype(o_ref.dtype)
            if n == 0:
                dep = att_rows(NF * R1, R2, False, pre) + ln_rows(xn_ref, ln1_scr, pre)
            else:
                dep = None

    @pl.when(i < NT)
    def _():
        x = x_ref[...].astype(F32)
        a = jnp.dot(att_scr[...], wo_scr[...], preferred_element_type=F32)
        h = (x + a.astype(BF16).astype(F32)).astype(BF16).astype(F32)
        h_scr[...] = h


@jax.jit
def pallas_sequential_preLN__sliding_local_dilated__dense_activation_relu__prompt_kernel(
    A_x, A_wqkv, A_wo, B_x, B_w1, B_w2):
    B, S, D = A_x.shape
    F = B_w1.shape[1]
    TS = 256
    FC = 512
    NC = 512
    NT = (B * S) // TS
    NV = D // 128
    NF = F // FC
    NN = D // NC
    R1 = 32
    R2 = TS - NF * R1
    x = A_x.reshape(B * S, D)
    kern = functools.partial(_kernel, TS=TS, D=D, F=F, FC=FC, NC=NC, NT=NT, R1=R1, R2=R2)
    hbm = pl.BlockSpec(memory_space=pltpu.MemorySpace.HBM)
    out = pl.pallas_call(
        kern,
        grid=(NT + 1,),
        in_specs=[
            hbm, hbm, hbm, hbm, hbm,
        ],
        out_specs=pl.BlockSpec((TS, D), lambda i: (jnp.maximum(i - 1, 0), 0)),
        out_shape=jax.ShapeDtypeStruct((B * S, D), A_x.dtype),
        scratch_shapes=[
            pltpu.VMEM((4, D, D), BF16),
            pltpu.VMEM((3, D, D), BF16),
            pltpu.VMEM((NV, D + H, 128), F32),
            pltpu.VMEM((D, D), BF16),
            pltpu.VMEM((NF, D, FC), BF16),
            pltpu.VMEM((NN, F, NC), BF16),
            pltpu.VMEM((3 * NV, TS + HALO, 128), F32),
            pltpu.VMEM((TS, D), BF16),
            pltpu.VMEM((TS, D), F32),
            pltpu.VMEM((TS, D), BF16),
            pltpu.VMEM((TS, F), BF16),
            pltpu.VMEM((TS, D), BF16),
            pltpu.VMEM((B * S, D), BF16),
            pltpu.SemaphoreType.DMA((4 + NF + NN + 4,)),
        ],
        compiler_params=pltpu.CompilerParams(
            dimension_semantics=("arbitrary",),
            vmem_limit_bytes=100 * 1024 * 1024,
        ),
    )(x, A_wqkv, A_wo, B_w1, B_w2)
    return out.reshape(B, S, D)
```

```python
import functools
import jax
import jax.numpy as jnp
from jax import lax
import jax.experimental.pallas as pl
import jax.experimental.pallas.tpu as pltpu

H = 32
WIN = 8
DIL = 2
HALO = 16
EPS = 1e-5
F32 = jnp.float32
BF16 = jnp.bfloat16


def _ln(x):
    m = jnp.mean(x, axis=-1, keepdims=True)
    xc = x - m
    v = jnp.mean(xc * xc, axis=-1, keepdims=True)
    return xc * lax.rsqrt(v + EPS)


def _kernel(x_hbm, wqkv_hbm, wo_hbm, w1_hbm, w2_hbm, o_ref,
            wraw_scr, wt_scr, stage_scr, wo_scr, w1_scr, w2_scr,
            qkv_scr, att_scr, h_scr, ln2_scr, h1_scr, ln1_scr, x_scr, sems, *, TS, D, F, FC, NC, NT, R1, R2):
    i = pl.program_id(0)
    Dh = D // H
    scale = Dh ** -0.5
    NV = D // 128
    G = 128 // H
    NF = F // FC
    NN = D // NC
    SS = Dh + 1

    def cp_qkv(p):
        return pltpu.make_async_copy(
            wqkv_hbm.at[:, pl.ds(pl.multiple_of(p * D, D), D)], wraw_scr.at[p], sems.at[p])

    def cp_wo():
        return pltpu.make_async_copy(wo_hbm, wraw_scr.at[3], sems.at[3])

    def cp_w1(f):
        return pltpu.make_async_copy(
            w1_hbm.at[:, pl.ds(pl.multiple_of(f * FC, FC), FC)], w1_scr.at[f], sems.at[4 + f])

    def cp_w2(n):
        return pltpu.make_async_copy(
            w2_hbm.at[:, pl.ds(pl.multiple_of(n * NC, NC), NC)], w2_scr.at[n], sems.at[4 + NF + n])

    XS = 4 + NF + NN

    def cp_x0():
        return pltpu.make_async_copy(x_hbm.at[pl.ds(0, TS), :], x_scr.at[pl.ds(0, TS), :], sems.at[XS])

    def cp_x1():
        return pltpu.make_async_copy(x_hbm.at[pl.ds(TS, TS), :], x_scr.at[pl.ds(TS, TS), :], sems.at[XS + 1])

    def cp_x2():
        return pltpu.make_async_copy(x_hbm.at[pl.ds(2 * TS, TS), :], x_scr.at[pl.ds(2 * TS, TS), :], sems.at[XS + 2])

    def cp_xr():
        n = (NT - 3) * TS
        return pltpu.make_async_copy(x_hbm.at[pl.ds(3 * TS, n), :], x_scr.at[pl.ds(3 * TS, n), :], sems.at[XS + 3])

    x_ref = x_scr.at[pl.ds(pl.multiple_of(jnp.minimum(i, NT - 1) * TS, TS), TS), :]
    xn_ref = x_scr.at[pl.ds(pl.multiple_of(jnp.minimum(i + 1, NT - 1) * TS, TS), TS), :]

    def perm_base(d):
        return (d // G) * 128 + (d % G) * H

    def att_rows(r0, nrows, masked, pres=None, RC=16):
        dep = None
        for c in range(nrows // RC):
            rr = r0 + c * RC
            pre = None if pres is None else pres[c]
            sc = scale if pre is None else scale + jnp.where(i < 0, pre, 0.0)
            q = [qkv_scr[j, pl.ds(HALO + rr, RC), :] * sc for j in range(NV)]
            logits = []
            for w in range(WIN):
                acc = None
                for j in range(NV):
                    kk = qkv_scr[NV + j, pl.ds(HALO + rr - DIL * w, RC), :]
                    t = q[j] * kk
                    acc = t if acc is None else acc + t
                acc = acc + pltpu.roll(acc, 64, 1)
                acc = acc + pltpu.roll(acc, 32, 1)
                if masked and w > 0:
                    row = rr + lax.broadcasted_iota(jnp.int32, (RC, 128), 0)
                    acc = jnp.where(row >= DIL * w, acc, -1e9)
                logits.append(acc)
            m = logits[0]
            for w in range(1, WIN):
                m = jnp.maximum(m, logits[w])
            es = [jnp.exp(l - m) for l in logits]
            den = es[0]
            for w in range(1, WIN):
                den = den + es[w]
            inv = 1.0 / den
            ps = [e * inv for e in es]
            for j in range(NV):
                acc = None
                for w in range(WIN):
                    vv = qkv_scr[2 * NV + j, pl.ds(HALO + rr - DIL * w, RC), :]
                    t = ps[w] * vv
                    acc = t if acc is None else acc + t
                att_scr[pl.ds(rr, RC), pl.ds(j * 128, 128)] = acc.astype(BF16)
                dep = acc if dep is None else dep + acc
        return dep

    def ln_rows(src_ref, dst_ref, pre=None, c_lo=0, c_hi=None):
        RC = 16
        dep = None
        for c in range(c_lo, TS // RC if c_hi is None else c_hi):
            xx = src_ref[pl.ds(c * RC, RC), :].astype(F32)
            m = jnp.mean(xx, axis=-1, keepdims=True)
            if pre is not None:
                m = m + jnp.where(i < 0, pre[:, 0:1], 0.0)
            xc = xx - m
            v = jnp.mean(xc * xc, axis=-1, keepdims=True)
            y = xc * lax.rsqrt(v + EPS)
            dst_ref[pl.ds(c * RC, RC), :] = y.astype(BF16)
            for j in range(NV):
                t = y[:, j * 128:(j + 1) * 128]
                dep = t if dep is None else dep + t
        return dep

    def tie(lhs, dep):
        if dep is None:
            return lhs
        z = jnp.where(i < 0, dep, 0.0)
        if z.shape[0] == 8:
            z = jnp.concatenate([z, z], axis=0)
        z = z.astype(lhs.dtype)
        top = lhs[0:16, :]
        top = jnp.concatenate([top[:, 0:128] + z, top[:, 128:]], axis=1)
        return jnp.concatenate([top, lhs[16:, :]], axis=0)

    @pl.when(i == 0)
    def _():
        cp_x0().start()
        cp_qkv(0).start()
        qkv_scr[:, pl.ds(0, HALO), :] = jnp.zeros((3 * NV, HALO, 128), F32)
        cp_x0().wait()
        cp_qkv(1).start()

        ln1_scr[...] = _ln(x_ref[...].astype(F32)).astype(BF16)

        def prep_part(p):
            for kb in range(NV):
                blk = wraw_scr[p, pl.ds(kb * 128, 128), :].astype(F32)
                blkt = blk.T
                for hh in range(H):
                    stage_scr[kb, pl.ds(hh * SS, Dh), :] = blkt[hh * Dh:(hh + 1) * Dh, :]
                for d in range(Dh):
                    rows = stage_scr[kb, pl.ds(d, H, stride=SS), :]
                    wt_scr[p, pl.ds(perm_base(d), H), pl.ds(kb * 128, 128)] = rows.astype(BF16)

        cp_qkv(0).wait()
        cp_qkv(2).start()
        prep_part(0)

        def qkv_first(p, carry):
            @pl.when(p < 2)
            def _():
                cp_qkv(p + 1).wait()

            @pl.when(p == 0)
            def _():
                cp_wo().start()
                cp_x1().start()

            @pl.when(p == 1)
            def _():
                cp_x2().start()
                for f in range(NF):
                    cp_w1(f).start()

            @pl.when(p == 2)
            def _():
                cp_wo().wait()
                for n in range(NN):
                    cp_w2(n).start()

            res = lax.dot_general(ln1_scr[...], wt_scr[p], (((1,), (1,)), ((), ())),
                                  preferred_element_type=F32)
            for j in range(NV):
                qkv_scr[p * NV + j, pl.ds(HALO, TS), :] = res[:, j * 128:(j + 1) * 128]
            prep_part(p + 1)
            return carry

        lax.fori_loop(0, 3, qkv_first, 0)

        def prep_wo(kb, carry):
            k0 = pl.multiple_of(kb * 128, 128)
            blkt = wraw_scr[3, :, pl.ds(k0, 128)].astype(F32)
            for hh in range(H):
                stage_scr[0, pl.ds(hh * SS, Dh), :] = blkt[hh * Dh:(hh + 1) * Dh, :]
            for d in range(Dh):
                rows = stage_scr[0, pl.ds(d, H, stride=SS), :]
                wo_scr[pl.ds(perm_base(d), H), pl.ds(k0, 128)] = rows.astype(BF16)
            return carry

        lax.fori_loop(0, NV, prep_wo, 0)
        cp_x1().wait()
        cp_xr().start()
        ln1_scr[...] = _ln(xn_ref[...].astype(F32)).astype(BF16)

    @pl.when(jnp.logical_and(i > 0, i < NT))
    def _():
        qkv_scr[:, pl.ds(0, HALO), :] = qkv_scr[:, pl.ds(TS, HALO), :]

    xp_ref = x_scr.at[pl.ds(pl.multiple_of(jnp.maximum(i - 1, 0) * TS, TS), TS), :]

    def out_proj():
        a = jnp.dot(att_scr[...], wo_scr[...], preferred_element_type=F32)
        h = (xp_ref[...].astype(F32) + a.astype(BF16).astype(F32)).astype(BF16).astype(F32)
        h_scr[...] = h

    @pl.when(jnp.logical_and(i > 0, i < NT))
    def _():
        out_proj()
        dep = None
        for p in range(3):
            res = lax.dot_general(tie(ln1_scr[...], dep), wt_scr[p], (((1,), (1,)), ((), ())),
                                  preferred_element_type=F32)
            for j in range(NV):
                qkv_scr[p * NV + j, pl.ds(HALO, TS), :] = res[:, j * 128:(j + 1) * 128]
            dep = ln_rows(h_scr, ln2_scr) if p == 0 else None

    @pl.when(i == NT)
    def _():
        out_proj()
        ln2_scr[...] = _ln(h_scr[...]).astype(BF16)

    @pl.when(i == 0)
    def _():
        att_rows(0, 16, True)
        att_rows(16, 16, False)

        def body(r, carry):
            att_rows(pl.multiple_of(r * 32, 32), 32, False)
            return carry
        lax.fori_loop(1, TS // 32, body, 0)

    @pl.when(i == 1)
    def _():
        for f in range(NF):
            cp_w1(f).wait()
        for n in range(NN):
            cp_w2(n).wait()
        cp_x2().wait()

    @pl.when(i == 2)
    def _():
        cp_xr().wait()

    @pl.when(i > 0)
    def _():
        def g16(v):
            return jnp.concatenate([v, v], axis=0)

        def fold(d):
            return d[0:8] + d[8:16]

        deps = [None, None]
        pre = None
        for f in range(NF):
            h1 = jnp.dot(tie(ln2_scr[...], deps[-2]), w1_scr[f], preferred_element_type=F32)
            h1_scr[:, pl.ds(f * FC, FC)] = jnp.maximum(h1, 0.0).astype(BF16)
            gates = [pre] + [h1[TS - 8:, t * 128:(t + 1) * 128] for t in range(3)]
            deps.append(att_rows(f * 32, 32, False, gates, RC=8))
            pre = h1[TS - 8:, FC - 128:]
        for n in range(NN):
            c0 = n * NC
            dd = deps[-2] if n == 0 else deps[-2] + deps[-1]
            t = jnp.dot(tie(h1_scr[...], dd), w2_scr[n], preferred_element_type=F32)
            o_ref[:, pl.ds(c0, NC)] = (
                h_scr[:, pl.ds(c0, NC)] + t.astype(BF16).astype(F32)).astype(o_ref.dtype)
            g = [pre] + [t[TS - 8:, k * 128:(k + 1) * 128] for k in range(3)]
            if n == 0:
                d = att_rows(NF * 32, 32, False, g, RC=8)
                for k in range(4):
                    d = d + fold(ln_rows(xn_ref, ln1_scr, g16(g[k]), 2 * k, 2 * k + 2))
                deps.append(d)
            else:
                ln_rows(xn_ref, ln1_scr, g16(g[0]), 8, 11)
                ln_rows(xn_ref, ln1_scr, g16(g[1]), 11, 14)
                ln_rows(xn_ref, ln1_scr, g16(g[2]), 14, 16)
            pre = t[TS - 8:, NC - 128:]


@jax.jit
def pallas_sequential_preLN__sliding_local_dilated__dense_activation_relu__prompt_kernel(
    A_x, A_wqkv, A_wo, B_x, B_w1, B_w2):
    B, S, D = A_x.shape
    F = B_w1.shape[1]
    TS = 256
    FC = 512
    NC = 512
    NT = (B * S) // TS
    NV = D // 128
    NF = F // FC
    NN = D // NC
    R1 = 32
    R2 = TS - NF * R1
    x = A_x.reshape(B * S, D)
    kern = functools.partial(_kernel, TS=TS, D=D, F=F, FC=FC, NC=NC, NT=NT, R1=R1, R2=R2)
    hbm = pl.BlockSpec(memory_space=pltpu.MemorySpace.HBM)
    out = pl.pallas_call(
        kern,
        grid=(NT + 1,),
        in_specs=[
            hbm, hbm, hbm, hbm, hbm,
        ],
        out_specs=pl.BlockSpec((TS, D), lambda i: (jnp.maximum(i - 1, 0), 0)),
        out_shape=jax.ShapeDtypeStruct((B * S, D), A_x.dtype),
        scratch_shapes=[
            pltpu.VMEM((4, D, D), BF16),
            pltpu.VMEM((4, D, D), BF16),
            pltpu.VMEM((NV, D + H, 128), F32),
            pltpu.VMEM((D, D), BF16),
            pltpu.VMEM((NF, D, FC), BF16),
            pltpu.VMEM((NN, F, NC), BF16),
            pltpu.VMEM((3 * NV, TS + HALO, 128), F32),
            pltpu.VMEM((TS, D), BF16),
            pltpu.VMEM((TS, D), F32),
            pltpu.VMEM((TS, D), BF16),
            pltpu.VMEM((TS, F), BF16),
            pltpu.VMEM((TS, D), BF16),
            pltpu.VMEM((B * S, D), BF16),
            pltpu.SemaphoreType.DMA((4 + NF + NN + 4,)),
        ],
        compiler_params=pltpu.CompilerParams(
            dimension_semantics=("arbitrary",),
            vmem_limit_bytes=100 * 1024 * 1024,
        ),
    )(x, A_wqkv, A_wo, B_w1, B_w2)
    return out.reshape(B, S, D)
```

```python
import functools
import jax
import jax.numpy as jnp
from jax import lax
import jax.experimental.pallas as pl
import jax.experimental.pallas.tpu as pltpu

H = 32
WIN = 8
DIL = 2
HALO = 16
EPS = 1e-5
F32 = jnp.float32
BF16 = jnp.bfloat16


def _ln(x):
    m = jnp.mean(x, axis=-1, keepdims=True)
    xc = x - m
    v = jnp.mean(xc * xc, axis=-1, keepdims=True)
    return xc * lax.rsqrt(v + EPS)


def _pk(x):
    return pltpu.bitcast(x, jnp.uint32)


def _upk(x):
    return pltpu.bitcast(x, BF16)


def _kernel(x_hbm, wqkv_hbm, wo_hbm, w1_hbm, w2_hbm, o_ref,
            wraw_scr, wt_scr, stage_scr, wo_scr, w1_scr, w2_scr,
            qkv_scr, att_scr, h_scr, ln2_scr, h1_scr, ln1_scr, x_scr, sems, *, TS, D, F, FC, NC, NT):
    i = pl.program_id(0)
    Dh = D // H
    scale = Dh ** -0.5
    NV = D // 128
    G = 128 // H
    NF = F // FC
    NN = D // NC
    SS = Dh + 1

    def cp_qkv(p):
        return pltpu.make_async_copy(
            wqkv_hbm.at[:, pl.ds(pl.multiple_of(p * D, D), D)], wraw_scr.at[p], sems.at[p])

    def cp_wo():
        return pltpu.make_async_copy(wo_hbm, wraw_scr.at[3], sems.at[3])

    def cp_w1(f):
        return pltpu.make_async_copy(
            w1_hbm.at[:, pl.ds(pl.multiple_of(f * FC, FC), FC)], w1_scr.at[f], sems.at[4 + f])

    def cp_w2(n):
        return pltpu.make_async_copy(
            w2_hbm.at[:, pl.ds(pl.multiple_of(n * NC, NC), NC)], w2_scr.at[n], sems.at[4 + NF + n])

    XS = 4 + NF + NN

    def cp_x0():
        return pltpu.make_async_copy(x_hbm.at[pl.ds(0, TS), :], x_scr.at[pl.ds(0, TS), :], sems.at[XS])

    def cp_x1():
        return pltpu.make_async_copy(x_hbm.at[pl.ds(TS, TS), :], x_scr.at[pl.ds(TS, TS), :], sems.at[XS + 1])

    def cp_x2():
        return pltpu.make_async_copy(x_hbm.at[pl.ds(2 * TS, TS), :], x_scr.at[pl.ds(2 * TS, TS), :], sems.at[XS + 2])

    def cp_xr():
        n = (NT - 3) * TS
        return pltpu.make_async_copy(x_hbm.at[pl.ds(3 * TS, n), :], x_scr.at[pl.ds(3 * TS, n), :], sems.at[XS + 3])

    x_ref = x_scr.at[pl.ds(pl.multiple_of(jnp.minimum(i, NT - 1) * TS, TS), TS), :]
    xn_ref = x_scr.at[pl.ds(pl.multiple_of(jnp.minimum(i + 1, NT - 1) * TS, TS), TS), :]

    def perm_base(d):
        return (d // G) * 128 + (d % G) * H

    def att_rows(r0, nrows, masked, pres=None, RC=16):
        dep = None
        for c in range(nrows // RC):
            rr = r0 + c * RC
            rh = rr // 2 if isinstance(rr, int) else pl.multiple_of(rr // 2, RC // 2)
            pre = None if pres is None else pres[c]
            sc = scale if pre is None else scale + jnp.where(i < 0, pre, 0.0)
            q = [qkv_scr[j, pl.ds(HALO + rr, RC), :] * sc for j in range(NV)]
            logits = []
            for w in range(WIN):
                acc = None
                for j in range(NV):
                    kk = qkv_scr[NV + j, pl.ds(HALO + rr - DIL * w, RC), :]
                    t = q[j] * kk
                    acc = t if acc is None else acc + t
                acc = acc + pltpu.roll(acc, 64, 1)
                acc = acc + pltpu.roll(acc, 32, 1)
                if masked and w > 0:
                    row = rr + lax.broadcasted_iota(jnp.int32, (RC, 128), 0)
                    acc = jnp.where(row >= DIL * w, acc, -1e9)
                logits.append(acc)
            m = logits[0]
            for w in range(1, WIN):
                m = jnp.maximum(m, logits[w])
            es = [jnp.exp(l - m) for l in logits]
            den = es[0]
            for w in range(1, WIN):
                den = den + es[w]
            inv = 1.0 / den
            ps = [e * inv for e in es]
            for j in range(NV):
                acc = None
                for w in range(WIN):
                    vv = qkv_scr[2 * NV + j, pl.ds(HALO + rr - DIL * w, RC), :]
                    t = ps[w] * vv
                    acc = t if acc is None else acc + t
                att_scr[pl.ds(rh, RC // 2), pl.ds(j * 128, 128)] = _pk(acc.astype(BF16))
                dep = acc if dep is None else dep + acc
        return dep

    def ln_rows(src_ref, dst_ref, pre=None, c_lo=0, c_hi=None):
        RC = 16
        dep = None
        for c in range(c_lo, TS // RC if c_hi is None else c_hi):
            xx = src_ref[pl.ds(c * RC, RC), :].astype(F32)
            m = jnp.mean(xx, axis=-1, keepdims=True)
            if pre is not None:
                m = m + jnp.where(i < 0, pre[:, 0:1], 0.0)
            xc = xx - m
            v = jnp.mean(xc * xc, axis=-1, keepdims=True)
            y = xc * lax.rsqrt(v + EPS)
            dst_ref[pl.ds(c * RC // 2, RC // 2), :] = _pk(y.astype(BF16))
            for j in range(NV):
                t = y[:, j * 128:(j + 1) * 128]
                dep = t if dep is None else dep + t
        return dep

    def tie(lhs, dep):
        if dep is None:
            return lhs
        z = jnp.where(i < 0, dep, 0.0)
        if z.shape[0] == 8:
            z = jnp.concatenate([z, z], axis=0)
        z = z.astype(lhs.dtype)
        top = lhs[0:16, :]
        top = jnp.concatenate([top[:, 0:128] + z, top[:, 128:]], axis=1)
        return jnp.concatenate([top, lhs[16:, :]], axis=0)

    @pl.when(i == 0)
    def _():
        cp_x0().start()
        cp_qkv(0).start()
        qkv_scr[:, pl.ds(0, HALO), :] = jnp.zeros((3 * NV, HALO, 128), F32)
        cp_x0().wait()
        cp_qkv(1).start()

        ln1_scr[...] = _pk(_ln(x_ref[...].astype(F32)).astype(BF16))

        def prep_part(p):
            for kb in range(NV):
                blk = wraw_scr[p, pl.ds(kb * 128, 128), :].astype(F32)
                blkt = blk.T
                for hh in range(H):
                    stage_scr[kb, pl.ds(hh * SS, Dh), :] = blkt[hh * Dh:(hh + 1) * Dh, :]
                for d in range(Dh):
                    rows = stage_scr[kb, pl.ds(d, H, stride=SS), :]
                    wt_scr[p, pl.ds(perm_base(d) // 2, H // 2), pl.ds(kb * 128, 128)] = _pk(rows.astype(BF16))

        cp_qkv(0).wait()
        cp_qkv(2).start()
        prep_part(0)

        def qkv_first(p, carry):
            @pl.when(p < 2)
            def _():
                cp_qkv(p + 1).wait()

            @pl.when(p == 0)
            def _():
                cp_wo().start()
                cp_x1().start()

            @pl.when(p == 1)
            def _():
                cp_x2().start()
                for f in range(NF):
                    cp_w1(f).start()

            @pl.when(p == 2)
            def _():
                cp_wo().wait()
                for n in range(NN):
                    cp_w2(n).start()

            res = lax.dot_general(_upk(ln1_scr[...]), _upk(wt_scr[p]), (((1,), (1,)), ((), ())),
                                  preferred_element_type=F32)
            for j in range(NV):
                qkv_scr[p * NV + j, pl.ds(HALO, TS), :] = res[:, j * 128:(j + 1) * 128]
            prep_part(p + 1)
            return carry

        lax.fori_loop(0, 3, qkv_first, 0)

        cp_x1().wait()
        cp_xr().start()
        ln1_scr[...] = _pk(_ln(xn_ref[...].astype(F32)).astype(BF16))

    @pl.when(jnp.logical_and(i > 0, i < NT))
    def _():
        qkv_scr[:, pl.ds(0, HALO), :] = qkv_scr[:, pl.ds(TS, HALO), :]

    xp_ref = x_scr.at[pl.ds(pl.multiple_of(jnp.maximum(i - 1, 0) * TS, TS), TS), :]

    def out_proj():
        a = jnp.dot(_upk(att_scr[...]), _upk(wo_scr[...]), preferred_element_type=F32)
        h = (xp_ref[...].astype(F32) + a.astype(BF16).astype(F32)).astype(BF16).astype(F32)
        h_scr[...] = h

    @pl.when(jnp.logical_and(i > 0, i < NT))
    def _():
        out_proj()
        dep = None
        for p in range(3):
            res = lax.dot_general(tie(_upk(ln1_scr[...]), dep), _upk(wt_scr[p]), (((1,), (1,)), ((), ())),
                                  preferred_element_type=F32)
            for j in range(NV):
                qkv_scr[p * NV + j, pl.ds(HALO, TS), :] = res[:, j * 128:(j + 1) * 128]
            if p == 0:
                d0 = None
                for k in range(NV):
                    gk = res[TS - 16:, k * 128:(k + 1) * 128]
                    dk = ln_rows(h_scr, ln2_scr, gk, 2 * k, 2 * k + 2)
                    d0 = dk if d0 is None else d0 + dk
                dep = None
            elif p == 1:
                dep = d0
            else:
                dep = None

    @pl.when(i == NT)
    def _():
        out_proj()
        ln2_scr[...] = _pk(_ln(h_scr[...]).astype(BF16))

    @pl.when(i == 0)
    def _():
        def prep_wo(kb):
            k0 = pl.multiple_of(kb * 128, 128)
            blkt = wraw_scr[3, :, pl.ds(k0, 128)].astype(F32)
            for hh in range(H):
                stage_scr[0, pl.ds(hh * SS, Dh), :] = blkt[hh * Dh:(hh + 1) * Dh, :]
            for d in range(Dh):
                rows = stage_scr[0, pl.ds(d, H, stride=SS), :]
                wo_scr[pl.ds(perm_base(d) // 2, H // 2), pl.ds(k0, 128)] = _pk(rows.astype(BF16))

        att_rows(0, 16, True)
        att_rows(16, 16, False)
        prep_wo(0)

        def body(r, carry):
            att_rows(pl.multiple_of(r * 32, 32), 32, False)
            prep_wo(r)
            return carry
        lax.fori_loop(1, TS // 32, body, 0)

    @pl.when(i == 1)
    def _():
        for f in range(NF):
            cp_w1(f).wait()
        for n in range(NN):
            cp_w2(n).wait()
        cp_x2().wait()

    @pl.when(i == 2)
    def _():
        cp_xr().wait()

    @pl.when(i > 0)
    def _():
        def g16(v):
            return jnp.concatenate([v, v], axis=0)

        def fold(d):
            return d[0:8] + d[8:16]

        deps = [None, None]
        pre = None
        for f in range(NF):
            h1 = jnp.dot(tie(_upk(ln2_scr[...]), deps[-2]), w1_scr[f], preferred_element_type=F32)
            h1_scr[:, pl.ds(f * FC, FC)] = _pk(jnp.maximum(h1, 0.0).astype(BF16))
            gates = [pre] + [h1[TS - 8:, t * 128:(t + 1) * 128] for t in range(3)]
            deps.append(att_rows(f * 32, 32, False, gates, RC=8))
            pre = h1[TS - 8:, FC - 128:]
        for n in range(NN):
            c0 = n * NC
            dd = deps[-2] if n == 0 else deps[-2] + deps[-1]
            t = jnp.dot(tie(_upk(h1_scr[...]), dd), w2_scr[n], preferred_element_type=F32)
            o_ref[:, pl.ds(c0, NC)] = (
                h_scr[:, pl.ds(c0, NC)] + t.astype(BF16).astype(F32)).astype(o_ref.dtype)
            g = [pre] + [t[TS - 8:, k * 128:(k + 1) * 128] for k in range(3)]
            if n == 0:
                d = att_rows(NF * 32, 32, False, g, RC=8)
                for k in range(4):
                    d = d + fold(ln_rows(xn_ref, ln1_scr, g16(g[k]), 2 * k, 2 * k + 2))
                deps.append(d)
            else:
                ln_rows(xn_ref, ln1_scr, g16(g[0]), 8, 11)
                ln_rows(xn_ref, ln1_scr, g16(g[1]), 11, 14)
                ln_rows(xn_ref, ln1_scr, g16(g[2]), 14, 16)
            pre = t[TS - 8:, NC - 128:]


@jax.jit
def pallas_sequential_preLN__sliding_local_dilated__dense_activation_relu__prompt_kernel(
    A_x, A_wqkv, A_wo, B_x, B_w1, B_w2):
    B, S, D = A_x.shape
    F = B_w1.shape[1]
    TS = 256
    assert B == 1 and D == 1024 and S % TS == 0 and S // TS >= 3 and F == 3584
    FC = 512
    NC = 512
    NT = (B * S) // TS
    NV = D // 128
    NF = F // FC
    NN = D // NC
    x = A_x.reshape(B * S, D)
    kern = functools.partial(_kernel, TS=TS, D=D, F=F, FC=FC, NC=NC, NT=NT)
    hbm = pl.BlockSpec(memory_space=pltpu.MemorySpace.HBM)
    out = pl.pallas_call(
        kern,
        grid=(NT + 1,),
        in_specs=[
            hbm, hbm, hbm, hbm, hbm,
        ],
        out_specs=pl.BlockSpec((TS, D), lambda i: (jnp.maximum(i - 1, 0), 0)),
        out_shape=jax.ShapeDtypeStruct((B * S, D), A_x.dtype),
        scratch_shapes=[
            pltpu.VMEM((4, D, D), BF16),
            pltpu.VMEM((4, D // 2, D), jnp.uint32),
            pltpu.VMEM((NV, D + H, 128), F32),
            pltpu.VMEM((D // 2, D), jnp.uint32),
            pltpu.VMEM((NF, D, FC), BF16),
            pltpu.VMEM((NN, F, NC), BF16),
            pltpu.VMEM((3 * NV, TS + HALO, 128), F32),
            pltpu.VMEM((TS // 2, D), jnp.uint32),
            pltpu.VMEM((TS, D), F32),
            pltpu.VMEM((TS // 2, D), jnp.uint32),
            pltpu.VMEM((TS // 2, F), jnp.uint32),
            pltpu.VMEM((TS // 2, D), jnp.uint32),
            pltpu.VMEM((B * S, D), BF16),
            pltpu.SemaphoreType.DMA((4 + NF + NN + 4,)),
        ],
        compiler_params=pltpu.CompilerParams(
            dimension_semantics=("arbitrary",),
            vmem_limit_bytes=100 * 1024 * 1024,
        ),
    )(x, A_wqkv, A_wo, B_w1, B_w2)
    return out.reshape(B, S, D)
```
